```python
import jax
import jax.numpy as jnp

def _softmax(x, axis=-1):
    return jax.nn.softmax(x, axis=axis)
def _gelu(x):
    return jax.nn.gelu(x, approximate=True)
def _silu(x):
    return jax.nn.silu(x)
def _sigmoid(x):
    return jax.nn.sigmoid(x)
def _layernorm(x, axis=-1, eps=1e-5):
    m = jnp.mean(x, axis=axis, keepdims=True)
    v = jnp.var(x, axis=axis, keepdims=True)
    return (x - m) / jnp.sqrt(v + eps)
def _scatter_add(tgt, idx, src, axis=0):
    return tgt.at[idx].add(src)
def _segment_sum(src, seg, n):
    return jax.ops.segment_sum(src, seg, n)
class _Rng:
    def __init__(self, key):
        self._k = key
    def _next(self):
        self._k, sub = jax.random.split(self._k)
        return sub
    def normal(self, shape):
        return jax.random.normal(self._next(), shape, dtype=jnp.bfloat16)
    def randint(self, lo, hi, shape):
        return jax.random.randint(self._next(), shape, lo, hi, dtype=jnp.int32)
    def uniform(self, shape, lo=0.0, hi=1.0):
        return jax.random.uniform(self._next(), shape, jnp.bfloat16, lo, hi)
    def permutation(self, n):
        return jax.random.permutation(self._next(), n)


kernel_name = 'concat_heads__sliding_local_dilated__ssm_conv_s5__prompt'

def setup_inputs():
    _rng = _Rng(jax.random.key(int.from_bytes(__import__("os").urandom(4), "little")))
    _w = (lambda a: (lambda t: t.astype(jnp.bfloat16) if jnp.issubdtype(t.dtype, jnp.floating) else t)(jnp.asarray(a)))
    def _A_setup():
        B, S, D = 1, 2048, 448
        return {
            "x": _w((lambda *s: _rng.normal(s) * 0.05)(B, S, D)),
            "wqkv": _w((lambda *s: _rng.normal(s) * 0.05)(D, 3 * D)),
            "wo": _w((lambda *s: _rng.normal(s) * 0.05)(D, D)),
        }
    _A_in = _A_setup()

    def _B_setup():
        B, S, D = 1, 2048, 448
        P = D
        Lambda_re = -0.5 * jnp.exp((lambda *s: _rng.normal(s) * 0.05)(P))
        Lambda_im = (lambda *s: _rng.normal(s) * 0.05)(P) * 1.0
        B_re = (lambda *s: _rng.normal(s) * 0.05)(P, D) * (D ** -0.5)
        B_im = (lambda *s: _rng.normal(s) * 0.05)(P, D) * (D ** -0.5)
        C_re = (lambda *s: _rng.normal(s) * 0.05)(D, P) * (P ** -0.5)
        C_im = (lambda *s: _rng.normal(s) * 0.05)(D, P) * (P ** -0.5)
        log_dt = (lambda *s: _rng.normal(s) * 0.05)(P) * 0.3 - 2.0
        Dskip = (lambda *s: _rng.normal(s) * 0.05)(D)
        return {
            "x": _w((lambda *s: _rng.normal(s) * 0.05)(B, S, D)),
            "Lambda_re": _w(Lambda_re),
            "Lambda_im": _w(Lambda_im),
            "B_re": _w(B_re),
            "B_im": _w(B_im),
            "C_re": _w(C_re),
            "C_im": _w(C_im),
            "log_dt": _w(log_dt),
            "Dskip": _w(Dskip),
        }
    _B_in = _B_setup()

    return {
        "A_x": _A_in["x"],
        "A_wqkv": _A_in["wqkv"],
        "A_wo": _A_in["wo"],
        "B_x": _B_in["x"],
        "B_Lambda_re": _B_in["Lambda_re"],
        "B_Lambda_im": _B_in["Lambda_im"],
        "B_B_re": _B_in["B_re"],
        "B_B_im": _B_in["B_im"],
        "B_C_re": _B_in["C_re"],
        "B_C_im": _B_in["C_im"],
        "B_log_dt": _B_in["log_dt"],
        "B_Dskip": _B_in["Dskip"],
    }

def reference(A_x, A_wqkv, A_wo, B_x, B_Lambda_re, B_Lambda_im, B_B_re, B_B_im, B_C_re, B_C_im, B_log_dt, B_Dskip):
    def _A_ref(x, wqkv, wo):
        B, S, D = x.shape
        H = 16; Dh = D // H
        W, dil = 8, 2
        qkv = (lambda x, *d: x.transpose(*d))((x @ wqkv).reshape(B, S, 3, H, Dh), 2, 0, 3, 1, 4)
        q, k, v = qkv[0], qkv[1], qkv[2]
        scale = Dh ** -0.5
        pos = jnp.arange(S)
        off = jnp.arange(W) * dil
        idx = pos[:, None] - off[None, :]
        mask = idx >= 0
        idx_c = jnp.where(mask, idx, 0).reshape(-1)
        kg = k[:, :, idx_c, :].reshape(B, H, S, W, Dh)
        vg = v[:, :, idx_c, :].reshape(B, H, S, W, Dh)
        logits = jnp.einsum("bhsd,bhswd->bhsw", q, kg) * scale
        logits = jnp.where(mask[None, None, :, :], logits, -1e9)
        attn = _softmax(logits, axis=-1)
        o = jnp.einsum("bhsw,bhswd->bhsd", attn, vg)
        return (lambda x, *d: x.transpose(*d))(o, 0, 2, 1, 3).reshape(B, S, D) @ wo

    def _B_ref(x, Lambda_re, Lambda_im, B_re, B_im, C_re, C_im, log_dt, Dskip):
        Bsz, L, H = x.shape
        Lam = Lambda_re + 1j * Lambda_im
        Bmat = B_re + 1j * B_im
        Cmat = C_re + 1j * C_im
        dt = jnp.exp(log_dt)
        Lam_bar = jnp.exp(dt * Lam)
        B_bar = ((Lam_bar - 1.0) / Lam)[:, None] * Bmat
        Bu = jnp.einsum("bld,pd->blp", x + 0j, B_bar)
        h = jnp.zeros_like(Bu[:, 0, :])
        hs = []
        for t in range(L):
            h = Lam_bar[None, :] * h + Bu[:, t, :]
            hs.append(h)
        hseq = jnp.stack(hs, 1)
        y = 2.0 * jnp.einsum("blp,dp->bld", hseq, Cmat).real + x * Dskip[None, None, :]
        return y

    a = _A_ref(A_x, A_wqkv, A_wo)
    b = _B_ref(B_x, B_Lambda_re, B_Lambda_im, B_B_re, B_B_im, B_C_re, B_C_im, B_log_dt, B_Dskip)
    return jnp.concatenate([a, b], axis=-1)
```

```python
import functools

import jax
import jax.numpy as jnp
import numpy as np
from jax import lax
import jax.experimental.pallas as pl
import jax.experimental.pallas.tpu as pltpu

S, D, H, DH, W = 2048, 448, 16, 28, 8
R = 512
NB = S // R
F32, BF16, U32 = jnp.float32, jnp.bfloat16, jnp.uint32
NT = (((1,), (1,)), ((), ()))
TN = (((0,), (0,)), ((), ()))
LW = (128, 128, 128, 64)


def _cmul(ar, ai, br, bi):
    return ar * br - ai * bi, ar * bi + ai * br


def _permute_rows(x_ref, xu_ref, xp_ref):
    xw = pltpu.bitcast(x_ref[...].T, U32)
    for k in range(4):
        xu_ref[k, :, 0:LW[k]] = xw[:, 128 * k:128 * k + LW[k]]
    for j in range(4):
        for k in range(4):
            w = xu_ref[k, pl.ds(j, 64, stride=4), 0:LW[k]]
            lo = pltpu.bitcast(w << 16, F32)
            hi = pltpu.bitcast(w & jnp.uint32(0xFFFF0000), F32)
            xp_ref[128 * j:128 * j + 64, 128 * k:128 * k + LW[k]] = lo.astype(BF16)
            xp_ref[128 * j + 64:128 * j + 128, 128 * k:128 * k + LW[k]] = hi.astype(BF16)


def _prep(wqkv_ref, wo_ref, lre_ref, lim_ref, cre_ref, cim_ref, ldt_ref, dsk_ref,
          wt_ref, wop_ref, bcat_ref, ccat_ref, lam_ref, tmp_ref, prev_ref, hc_ref):
    wT = wqkv_ref[...].astype(F32).T
    for k in range(4):
        tmp_ref[k, :, 0:LW[k]] = wT[:, 128 * k:128 * k + LW[k]]
    for part in range(3):
        for d in range(DH):
            for k in range(4):
                v = tmp_ref[k, pl.ds(part * D + d, H, stride=DH), 0:LW[k]]
                r0 = part * D + d * H
                wt_ref[r0:r0 + H, 128 * k:128 * k + LW[k]] = v.astype(BF16)
    wo = wo_ref[...].astype(F32)
    for k in range(4):
        tmp_ref[k, 0:D, 0:LW[k]] = wo[:, 128 * k:128 * k + LW[k]]
    for d in range(DH):
        for k in range(4):
            v = tmp_ref[k, pl.ds(d, H, stride=DH), 0:LW[k]]
            wop_ref[d * H:(d + 1) * H, 128 * k:128 * k + LW[k]] = v.astype(BF16)
    lr = lre_ref[...].astype(F32).reshape(1, D)
    li = lim_ref[...].astype(F32).reshape(1, D)
    dt = jnp.exp(ldt_ref[...].astype(F32).reshape(1, D)).astype(BF16).astype(F32)
    mag = jnp.exp(dt * lr)
    ar = mag * jnp.cos(dt * li)
    ai = mag * jnp.sin(dt * li)
    den = lr * lr + li * li
    nr, ni = ar - 1.0, ai
    cr = (nr * lr + ni * li) / den
    ci = (ni * lr - nr * li) / den
    c_re = cre_ref[...].astype(F32)
    c_im = cim_ref[...].astype(F32)
    pr = 2.0 * (c_re * cr - c_im * ci)
    pi = -2.0 * (c_re * ci + c_im * cr)
    ccat_ref[0:64, :] = jnp.zeros((64, 2 * D), BF16)
    ccat_ref[64:512, 0:384] = pr[:, 0:384].astype(BF16)
    ccat_ref[64:512, 384:768] = pi[:, 0:384].astype(BF16)
    ccat_ref[64:512, 768:896] = jnp.concatenate([pr[:, 384:448], pi[:, 384:448]], axis=1).astype(BF16)
    ar = jnp.concatenate([ar, ar[:, 384:448]], axis=1)
    ai = jnp.concatenate([ai, -ai[:, 384:448]], axis=1)
    dsk = jnp.concatenate([jnp.zeros((1, 64), F32), dsk_ref[...].astype(F32).reshape(1, D)], axis=1)
    bc = lambda v: jnp.broadcast_to(v, (8, 512))
    lam_ref[0] = bc(ar)
    lam_ref[1] = bc(ai)
    p2 = _cmul(ar, ai, ar, ai)
    p4 = _cmul(*p2, *p2)
    p8 = _cmul(*p4, *p4)
    p16 = _cmul(*p8, *p8)
    p32 = _cmul(*p16, *p16)
    sub = lax.broadcasted_iota(jnp.int32, (8, 512), 0)
    for n, (p, sh) in enumerate(((p8, 1), (p16, 2), (p32, 4))):
        lam_ref[2 + 2 * n] = jnp.where(sub >= sh, bc(p[0]), 0.0)
        lam_ref[3 + 2 * n] = jnp.where(sub >= sh, bc(p[1]), 0.0)
    qr, qi = bc(p8[0]), bc(p8[1])
    for p, bit in ((p8, 1), (p16, 2), (p32, 4)):
        mr, mi = _cmul(qr, qi, bc(p[0]), bc(p[1]))
        on = (sub & bit) != 0
        qr = jnp.where(on, mr, qr)
        qi = jnp.where(on, mi, qi)
    lam_ref[8] = qr
    lam_ref[9] = qi
    lam_ref[10] = bc(dsk)
    prev_ref[...] = jnp.zeros(prev_ref.shape, F32)
    hc_ref[...] = jnp.zeros(hc_ref.shape, F32)


def _shifted(qkv_ref, prev_ref, base, r0, c63, c62):
    cur = [qkv_ref[base + r0:base + r0 + 8, 128 * j:128 * j + 128] for j in range(4)]
    pr0 = base - D + r0
    prv = [prev_ref[pr0:pr0 + 8, 128 * j:128 * j + 128] for j in range(4)]
    for j in range(4):
        prev_ref[pr0:pr0 + 8, 128 * j:128 * j + 128] = pltpu.roll(cur[j], 64, 1)
    r1 = [pltpu.roll(jnp.where(c63, prv[j], cur[j]), 1, 1) for j in range(4)]
    r2 = [pltpu.roll(jnp.where(c62, prv[j], cur[j]), 2, 1) for j in range(1, 4)]
    return r2 + r1 + cur


def _attention(qkv_ref, prev_ref, ot_ref, first):
    lane = lax.broadcasted_iota(jnp.int32, (8, 128), 1) & 63
    c63, c62 = lane >= 63, lane >= 62
    lim1 = jnp.where(first, 1, 0)
    lim2 = jnp.where(first, 2, 0)
    bad1, bad2 = lane < lim1, lane < lim2
    scale = DH ** -0.5
    for hg in range(2):
        acc = [[None] * W for _ in range(4)]
        for d in range(DH):
            r0 = d * H + hg * 8
            ks = _shifted(qkv_ref, prev_ref, D, r0, c63, c62)
            for j in range(4):
                q = qkv_ref[r0:r0 + 8, 128 * j:128 * j + 128]
                for w in range(W):
                    t = q * ks[7 + j - w]
                    acc[j][w] = t if d == 0 else acc[j][w] + t
        p = []
        for j in range(4):
            l = []
            for w in range(W):
                v = acc[j][w] * scale
                if j - w < -4:
                    v = jnp.where(bad2, -1e9, v)
                elif j - w < 0:
                    v = jnp.where(bad1, -1e9, v)
                l.append(v)
            m = functools.reduce(jnp.maximum, l)
            e = [jnp.exp(v - m) for v in l]
            inv = 1.0 / functools.reduce(jnp.add, e)
            p.append([v * inv for v in e])
        for d in range(DH):
            r0 = d * H + hg * 8
            vs = _shifted(qkv_ref, prev_ref, 2 * D, r0, c63, c62)
            for j in range(4):
                o = p[j][0] * vs[7 + j]
                for w in range(1, W):
                    o = o + p[j][w] * vs[7 + j - w]
                ot_ref[r0:r0 + 8, 128 * j:128 * j + 128] = o


def _scan(bu_ref, lam_ref, hc_ref, h_ref):
    sub = lax.broadcasted_iota(jnp.int32, (8, 128), 0)
    for k in range(4):
        ln = slice(128 * k, 128 * k + 128)
        lam = [lam_ref[n, :, ln] for n in range(10)]
        ar = jnp.tile(lam[0], (8, 1))
        ai = jnp.tile(lam[1], (8, 1))
        if k < 3:
            cre, cim = ln, slice(384 + 128 * k, 512 + 128 * k)
            ld = lambda jj: (bu_ref[64 * jj:64 * jj + 64, cre], bu_ref[64 * jj:64 * jj + 64, cim])
        else:
            cre = slice(768, 896)

            def ld(jj):
                z = bu_ref[64 * jj:64 * jj + 64, cre]
                return z, pltpu.roll(z, 64, 1)
        sr, si = ld(0)
        for jj in range(1, 8):
            br, bi = ld(jj)
            sr, si = ar * sr - ai * si + br, ar * si + ai * sr + bi
        pr, pi = hc_ref[0, :, ln], hc_ref[1, :, ln]
        inr, ini = [], []
        for cg in range(8):
            er, ei = sr[8 * cg:8 * cg + 8], si[8 * cg:8 * cg + 8]
            for n, sh in enumerate((1, 2, 4)):
                tr, ti = pltpu.roll(er, sh, 0), pltpu.roll(ei, sh, 0)
                mr, mi = _cmul(lam[2 + 2 * n], lam[3 + 2 * n], tr, ti)
                er, ei = er + mr, ei + mi
            br = jnp.broadcast_to(pr[7:8], (8, 128))
            bi = jnp.broadcast_to(pi[7:8], (8, 128))
            mr, mi = _cmul(lam[8], lam[9], br, bi)
            er, ei = er + mr, ei + mi
            inr.append(jnp.where(sub == 0, br, pltpu.roll(er, 1, 0)))
            ini.append(jnp.where(sub == 0, bi, pltpu.roll(ei, 1, 0)))
            pr, pi = er, ei
        hc_ref[0, :, ln] = pr
        hc_ref[1, :, ln] = pi
        sr, si = jnp.concatenate(inr, 0), jnp.concatenate(ini, 0)
        for jj in range(8):
            br, bi = ld(jj)
            sr, si = ar * sr - ai * si + br, ar * si + ai * sr + bi
            h_ref[64 * jj:64 * jj + 64, cre] = sr.astype(BF16)
            if k < 3:
                h_ref[64 * jj:64 * jj + 64, cim] = si.astype(BF16)


def _kernel(xa_hbm, wqkv_hbm, wo_hbm, xb_hbm, lre_ref, lim_ref, bre_hbm, bim_hbm, cre_hbm, cim_hbm,
            ldt_ref, dsk_ref, out_ref,
            xa_ref, xb_ref, wqkv_ref, wo_ref, cre_ref, cim_ref, isem, xsem,
            wt_ref, wop_ref, bcat_ref, ccat_ref, lam_ref, tmp_ref, prev_ref, hc_ref,
            xau_ref, xbu_ref, xap_ref, xbp_ref, qkv_ref, ot_ref, bu_ref, h_ref, stage_ref, sem):
    i = pl.program_id(0)
    slot = i % 2

    def out_copy(blk, sl, k):
        return pltpu.make_async_copy(
            stage_ref.at[sl, k],
            out_ref.at[pl.ds(pl.multiple_of(blk * R, R), R), pl.ds(128 * k, 128)],
            sem.at[sl, k])

    def x_copies(blk, sl):
        cols = pl.ds(pl.multiple_of(blk * R, R), R)
        return (pltpu.make_async_copy(xb_hbm.at[:, cols], xb_ref.at[sl], xsem.at[sl, 0]),
                pltpu.make_async_copy(xa_hbm.at[:, cols], xa_ref.at[sl], xsem.at[sl, 1]))

    @pl.when(i == 0)
    def _():
        cps = [
            pltpu.make_async_copy(wqkv_hbm, wqkv_ref, isem.at[0]),
            pltpu.make_async_copy(wo_hbm, wo_ref, isem.at[1]),
            pltpu.make_async_copy(cre_hbm, cre_ref, isem.at[2]),
            pltpu.make_async_copy(cim_hbm, cim_ref, isem.at[3]),
            pltpu.make_async_copy(bre_hbm.at[0:384], bcat_ref.at[0:384], isem.at[4]),
            pltpu.make_async_copy(bim_hbm.at[0:384], bcat_ref.at[384:768], isem.at[5]),
            pltpu.make_async_copy(bre_hbm.at[384:448], bcat_ref.at[768:832], isem.at[6]),
            pltpu.make_async_copy(bim_hbm.at[384:448], bcat_ref.at[832:896], isem.at[7]),
        ]
        for c in cps:
            c.start()
        for c in x_copies(0, 0):
            c.start()
        for c in cps:
            c.wait()
        _prep(wqkv_ref, wo_ref, lre_ref, lim_ref, cre_ref, cim_ref, ldt_ref, dsk_ref,
              wt_ref, wop_ref, bcat_ref, ccat_ref, lam_ref, tmp_ref, prev_ref, hc_ref)

    @pl.when(i >= 2)
    def _():
        for k in range(7):
            out_copy(i - 2, slot, k).wait()

    @pl.when(i + 1 < NB)
    def _():
        for c in x_copies(i + 1, 1 - slot):
            c.start()

    for c in x_copies(i, slot):
        c.wait()

    _permute_rows(xb_ref.at[slot], xbu_ref, xbp_ref)
    bu_ref[...] = lax.dot_general(xbp_ref[...], bcat_ref[...], NT, preferred_element_type=F32)
    _permute_rows(xa_ref.at[slot], xau_ref, xap_ref)
    qkv_ref[0:2 * D] = lax.dot_general(wt_ref[0:2 * D], xap_ref[...], NT, preferred_element_type=F32)
    _scan(bu_ref, lam_ref, hc_ref, h_ref)
    qkv_ref[2 * D:] = lax.dot_general(wt_ref[2 * D:], xap_ref[...], NT, preferred_element_type=F32)
    y = lax.dot_general(h_ref[...], ccat_ref[...], NT, preferred_element_type=F32)
    _attention(qkv_ref, prev_ref, ot_ref, i == 0)
    a = lax.dot_general(ot_ref[...].astype(BF16), wop_ref[...], TN, preferred_element_type=F32)

    lo = lax.broadcasted_iota(jnp.int32, (64, 128), 1) < 64
    for j in range(4):
        rot = []
        for k in range(4):
            w = xbu_ref[k, pl.ds(j, 64, stride=4), 0:LW[k]]
            if k == 3:
                w = jnp.concatenate([w, w], axis=1)
            rot.append(pltpu.roll(w, 64, 1))
        for k in range(4):
            w = rot[0] if k == 0 else jnp.where(lo, rot[k - 1], rot[k])
            dk = lam_ref[10, 0:1, 128 * k:128 * k + 128]
            for par in range(2):
                jj = 2 * j + par
                xv = pltpu.bitcast((w << 16) if par == 0 else (w & jnp.uint32(0xFFFF0000)), F32)
                b = y[64 * jj:64 * jj + 64, 128 * k:128 * k + 128] + xv * dk
                if k == 0:
                    a3 = a[64 * jj:64 * jj + 64, 384:448]
                    b = jnp.where(lo, jnp.concatenate([a3, a3], axis=1), b)
                stage_ref[slot, 3 + k, pl.ds(jj, 64, stride=8), :] = b
        for par in range(2):
            jj = 2 * j + par
            for k in range(3):
                stage_ref[slot, k, pl.ds(jj, 64, stride=8), :] = a[64 * jj:64 * jj + 64, 128 * k:128 * k + 128]

    for k in range(7):
        out_copy(i, slot, k).start()

    @pl.when(i == NB - 1)
    def _():
        for k in range(7):
            out_copy(i - 1, 1 - slot, k).wait()
        for k in range(7):
            out_copy(i, slot, k).wait()


def _call(A_x, A_wqkv, A_wo, B_x, lre, lim, bre, bim, cre, cim, ldt, dsk, interpret=False):
    full = lambda a: pl.BlockSpec(a.shape, lambda i: (0,) * a.ndim)
    hbm = pl.BlockSpec(memory_space=pltpu.HBM)
    out = pl.pallas_call(
        _kernel,
        grid=(NB,),
        in_specs=[hbm, hbm, hbm, hbm, full(lre), full(lim), hbm, hbm, hbm, hbm, full(ldt), full(dsk)],
        out_specs=hbm,
        out_shape=jax.ShapeDtypeStruct((S, 2 * D), F32),
        scratch_shapes=[
            pltpu.VMEM((2, D, R), BF16),
            pltpu.VMEM((2, D, R), BF16),
            pltpu.VMEM((D, 3 * D), BF16),
            pltpu.VMEM((D, D), BF16),
            pltpu.VMEM((D, D), BF16),
            pltpu.VMEM((D, D), BF16),
            pltpu.SemaphoreType.DMA((8,)),
            pltpu.SemaphoreType.DMA((2, 2)),
            pltpu.VMEM((3 * D, D), BF16),
            pltpu.VMEM((D, D), BF16),
            pltpu.VMEM((2 * D, D), BF16),
            pltpu.VMEM((512, 2 * D), BF16),
            pltpu.VMEM((11, 8, 512), F32),
            pltpu.VMEM((4, 3 * D, 128), F32),
            pltpu.VMEM((2 * D, R), F32),
            pltpu.VMEM((2, 8, 512), F32),
            pltpu.VMEM((4, R // 2, 128), U32),
            pltpu.VMEM((4, R // 2, 128), U32),
            pltpu.VMEM((R, D), BF16),
            pltpu.VMEM((R, D), BF16),
            pltpu.VMEM((3 * D, R), F32),
            pltpu.VMEM((D, R), F32),
            pltpu.VMEM((R, 2 * D), F32),
            pltpu.VMEM((R, 2 * D), BF16),
            pltpu.VMEM((2, 7, R, 128), F32),
            pltpu.SemaphoreType.DMA((2, 7)),
        ],
        compiler_params=pltpu.CompilerParams(
            dimension_semantics=("arbitrary",), vmem_limit_bytes=100 * 2**20),
        interpret=interpret,
        name="fused",
    )(A_x.reshape(S, D).T, A_wqkv, A_wo, B_x.reshape(S, D).T, lre, lim, bre, bim, cre, cim, ldt, dsk)
    return out.reshape(1, S, 2 * D)


@jax.jit
def pallas_concat_heads__sliding_local_dilated__ssm_conv_s5__prompt_kernel(
    A_x, A_wqkv, A_wo, B_x, B_Lambda_re, B_Lambda_im, B_B_re, B_B_im, B_C_re, B_C_im, B_log_dt, B_Dskip,
):
    return _call(A_x, A_wqkv, A_wo, B_x, B_Lambda_re, B_Lambda_im, B_B_re, B_B_im, B_C_re, B_C_im,
                 B_log_dt, B_Dskip)
```

```python
import functools

import jax
import jax.numpy as jnp
from jax import lax
import jax.experimental.pallas as pl
import jax.experimental.pallas.tpu as pltpu

S, D, H, DH, W = 2048, 448, 16, 28, 8
R = 512
NB = S // R
PM = 112
F32, BF16, U32 = jnp.float32, jnp.bfloat16, jnp.uint32
NT = (((1,), (1,)), ((), ()))
LW = (128, 128, 128, 64)


def _cmul(ar, ai, br, bi):
    return ar * br - ai * bi, ar * bi + ai * br


def _permute_rows(x_ref, xu_ref, xp_ref):
    xw = pltpu.bitcast(x_ref[...].T, U32)
    for k in range(4):
        xu_ref[k, :, 0:LW[k]] = xw[:, 128 * k:128 * k + LW[k]]
    for j in range(4):
        for k in range(4):
            w = xu_ref[k, pl.ds(j, 64, stride=4), 0:LW[k]]
            lo = pltpu.bitcast(w << 16, F32)
            hi = pltpu.bitcast(w & jnp.uint32(0xFFFF0000), F32)
            xp_ref[k, 128 * j:128 * j + 64, 0:LW[k]] = lo.astype(BF16)
            xp_ref[k, 128 * j + 64:128 * j + 128, 0:LW[k]] = hi.astype(BF16)


def _prep_wqkv(wqkv_ref, wt_ref, tmp_ref):
    wT = wqkv_ref[...].astype(F32).T
    for k in range(4):
        tmp_ref[k, :, 0:LW[k]] = wT[:, 128 * k:128 * k + LW[k]]
    for part in range(3):
        for d in range(DH):
            for k in range(4):
                v = tmp_ref[k, pl.ds(part * D + d, H, stride=DH), 0:LW[k]]
                r0 = part * D + d * H
                wt_ref[k, r0:r0 + H, 0:LW[k]] = v.astype(BF16)


def _prep_wo(wo_ref, wot_ref, tmp_ref, tmp2_ref):
    wo = wo_ref[...].astype(F32)
    for k in range(4):
        tmp_ref[k, :, 0:LW[k]] = wo[:, 128 * k:128 * k + LW[k]]
    for d in range(DH):
        for k in range(4):
            tmp2_ref[d * H:(d + 1) * H, 128 * k:128 * k + LW[k]] = tmp_ref[k, pl.ds(d, H, stride=DH), 0:LW[k]]
    wot = tmp2_ref[...].T.astype(BF16)
    for k in range(4):
        wot_ref[k, :, 0:LW[k]] = wot[:, 128 * k:128 * k + LW[k]]


def _prep_lam(lre_ref, lim_ref, ldt_ref, dsk_ref, lam_ref):
    lr = lre_ref[...].astype(F32).reshape(1, D)
    li = lim_ref[...].astype(F32).reshape(1, D)
    dt = jnp.exp(ldt_ref[...].astype(F32).reshape(1, D)).astype(BF16).astype(F32)
    mag = jnp.exp(dt * lr)
    ar = mag * jnp.cos(dt * li)
    ai = mag * jnp.sin(dt * li)
    den = lr * lr + li * li
    nr, ni = ar - 1.0, ai
    cr = (nr * lr + ni * li) / den
    ci = (ni * lr - nr * li) / den
    ar = jnp.concatenate([ar, ar[:, 384:448]], axis=1)
    ai = jnp.concatenate([ai, -ai[:, 384:448]], axis=1)
    dsk = jnp.concatenate([jnp.zeros((1, 64), F32), dsk_ref[...].astype(F32).reshape(1, D)], axis=1)
    bc = lambda v: jnp.broadcast_to(v, (8, 512))
    lam_ref[0] = bc(ar)
    lam_ref[1] = bc(ai)
    p2 = _cmul(ar, ai, ar, ai)
    p4 = _cmul(*p2, *p2)
    p8 = _cmul(*p4, *p4)
    p16 = _cmul(*p8, *p8)
    p32 = _cmul(*p16, *p16)
    p64 = _cmul(*p32, *p32)
    p128 = _cmul(*p64, *p64)
    p256 = _cmul(*p128, *p128)
    sub = lax.broadcasted_iota(jnp.int32, (8, 512), 0)
    for n, (p, sh) in enumerate(((p64, 1), (p128, 2), (p256, 4))):
        lam_ref[2 + 2 * n] = jnp.where(sub >= sh, bc(p[0]), 0.0)
        lam_ref[3 + 2 * n] = jnp.where(sub >= sh, bc(p[1]), 0.0)
    lam_ref[8] = bc(p8[0])
    lam_ref[9] = bc(p8[1])
    lam_ref[10] = bc(dsk)
    return 2.0 * cr, 2.0 * ci


def _prep_c(coef, cre_ref, cim_ref, ccat_ref):
    cr2, ci2 = coef
    for r in range(0, D, 32):
        c_re = cre_ref[r:r + 32, :].astype(F32)
        c_im = cim_ref[r:r + 32, :].astype(F32)
        pr = c_re * cr2 - c_im * ci2
        pi = -(c_re * ci2 + c_im * cr2)
        for k in range(3):
            ccat_ref[2 * k, r:r + 32] = pr[:, 128 * k:128 * k + 128].astype(BF16)
            ccat_ref[2 * k + 1, r:r + 32] = pi[:, 128 * k:128 * k + 128].astype(BF16)
        ccat_ref[6, r:r + 32] = jnp.concatenate([pr[:, 384:448], pi[:, 384:448]], axis=1).astype(BF16)


def _extend(qkv_ref, prev_ref, ext_ref, part, hg, first):
    lane = lax.broadcasted_iota(jnp.int32, (8, 128), 1) & 63
    c63, c62 = lane >= 63, lane >= 62
    for d in range(DH):
        r0 = d * H + hg * 8
        for j in range(4):
            ln = slice(128 * j, 128 * j + 128)
            cur = qkv_ref[1 + part][r0:r0 + 8, ln]
            ext_ref[7 + j, r0:r0 + 8] = cur
            prv = 0.0 if first else prev_ref[part, r0:r0 + 8, ln]
            prev_ref[part, r0:r0 + 8, ln] = pltpu.roll(cur, 64, 1)
            ext_ref[3 + j, r0:r0 + 8] = pltpu.roll(jnp.where(c63, prv, cur), 1, 1)
            if j:
                ext_ref[j - 1, r0:r0 + 8] = pltpu.roll(jnp.where(c62, prv, cur), 2, 1)
        yield


def _window(ext_ref, r0, j0):
    return {m: ext_ref[m + 7, pl.ds(r0, 8)] for m in range(j0 - 7, j0 + 2)}


def _logits(qkv_ref, ext_ref, p_ref, j0, first):
    lane = lax.broadcasted_iota(jnp.int32, (8, 128), 1) & 63
    scale = DH ** -0.5
    for hg in range(2):
        acc = {}
        for d in range(DH):
            r0 = d * H + hg * 8
            ks = _window(ext_ref, r0, j0)
            for j in (j0, j0 + 1):
                q = qkv_ref[0][r0:r0 + 8, 128 * j:128 * j + 128]
                for w in range(W):
                    t = q * ks[j - w]
                    acc[j, w] = t if d == 0 else acc[j, w] + t
            if d % 2:
                yield
        for j in (j0, j0 + 1):
            l = []
            for w in range(W):
                v = acc[j, w] * scale
                if first and j - w < 0:
                    v = jnp.where(lane < (2 if j - w < -4 else 1), -1e9, v)
                l.append(v)
            m = functools.reduce(jnp.maximum, l)
            e = [jnp.exp(v - m) for v in l]
            inv = 1.0 / functools.reduce(jnp.add, e)
            for w in range(W):
                p_ref[hg, j * W + w] = e[w] * inv
            yield


def _values(ext_ref, p_ref, ot_ref, j0):
    for hg in range(2):
        p = {(j, w): p_ref[hg, j * W + w] for j in (j0, j0 + 1) for w in range(W)}
        for d in range(DH):
            r0 = d * H + hg * 8
            vs = _window(ext_ref, r0, j0)
            for j in (j0, j0 + 1):
                o = p[j, 0] * vs[j]
                for w in range(1, W):
                    o = o + p[j, w] * vs[j - w]
                ot_ref[j, r0:r0 + 8] = o
            if d % 2:
                yield


def _scan(bu_ref, lam_ref, hc_ref, h_ref, e_ref, k, first):
    sub = lax.broadcasted_iota(jnp.int32, (8, 128), 0)
    ln = slice(128 * k, 128 * k + 128)
    lam = [lam_ref[n, :, ln] for n in range(10)]
    ar = jnp.tile(lam[0], (8, 1))
    ai = jnp.tile(lam[1], (8, 1))
    if k < 3:
        cre, cim = slice(256 * k, 256 * k + 128), slice(256 * k + 128, 256 * k + 256)
        ld = lambda jj: (bu_ref[64 * jj:64 * jj + 64, cre], bu_ref[64 * jj:64 * jj + 64, cim])
    else:
        cre = slice(768, 896)

        def ld(jj):
            z = bu_ref[64 * jj:64 * jj + 64, cre]
            return z, pltpu.roll(z, 64, 1)
    sr, si = ld(0)
    for jj in range(1, 8):
        br, bi = ld(jj)
        sr, si = ar * sr - ai * si + br, ar * si + ai * sr + bi
        yield
    for cg in range(8):
        e_ref[k, 0, 9 * cg:9 * cg + 8] = sr[8 * cg:8 * cg + 8]
        e_ref[k, 1, 9 * cg:9 * cg + 8] = si[8 * cg:8 * cg + 8]
    es = [(e_ref[k, 0, pl.ds(n, 8, stride=9)], e_ref[k, 1, pl.ds(n, 8, stride=9)]) for n in range(8)]
    er, ei = es[0]
    for n in range(1, 8):
        mr, mi = _cmul(lam[8], lam[9], er, ei)
        er, ei = es[n][0] + mr, es[n][1] + mi
    yield
    if first:
        pr = pi = 0.0
    else:
        pr, pi = pltpu.roll(hc_ref[0, :, ln], 1, 0), pltpu.roll(hc_ref[1, :, ln], 1, 0)
    er = jnp.where(sub == 0, pr, pltpu.roll(er, 1, 0))
    ei = jnp.where(sub == 0, pi, pltpu.roll(ei, 1, 0))
    for n, sh in enumerate((1, 2, 4)):
        tr, ti = pltpu.roll(er, sh, 0), pltpu.roll(ei, sh, 0)
        mr, mi = _cmul(lam[2 + 2 * n], lam[3 + 2 * n], tr, ti)
        er, ei = er + mr, ei + mi
    yield
    for n in range(8):
        e_ref[k, 0, pl.ds(n, 8, stride=9)] = er
        e_ref[k, 1, pl.ds(n, 8, stride=9)] = ei
        mr, mi = _cmul(lam[8], lam[9], er, ei)
        er, ei = es[n][0] + mr, es[n][1] + mi
    hc_ref[0, :, ln] = er
    hc_ref[1, :, ln] = ei
    yield
    sr = jnp.concatenate([e_ref[k, 0, 9 * cg:9 * cg + 8] for cg in range(8)], 0)
    si = jnp.concatenate([e_ref[k, 1, 9 * cg:9 * cg + 8] for cg in range(8)], 0)
    for jj in range(8):
        br, bi = ld(jj)
        sr, si = ar * sr - ai * si + br, ar * si + ai * sr + bi
        h_ref[2 * k, 64 * jj:64 * jj + 64] = sr.astype(BF16)
        if k < 3:
            h_ref[2 * k + 1, 64 * jj:64 * jj + 64] = si.astype(BF16)
        yield


def _chain(*gens):
    for g in gens:
        yield from g


def _mix(pieces, gen, n_units, skip=0):
    done = 0
    for n, piece in enumerate(pieces):
        piece()
        target = (n + 1 - skip) * n_units // (len(pieces) - skip)
        while done < target:
            next(gen, None)
            done += 1


def _store_tile(oa_ref, oy_ref, xu_ref, lam_ref, stage_ref, t):
    if t < 3:
        o = oa_ref[128 * t:128 * t + 128, :]
    elif t == 3:
        o = jnp.concatenate([oa_ref[384:448, :], oy_ref[0:64, :]], axis=0)
    else:
        o = oy_ref[128 * t - D:128 * t - D + 128, :]
    o = o.T
    lo = lax.broadcasted_iota(jnp.int32, (64, 128), 1) < 64
    for j in range(4):
        if t >= 3:
            k = t - 3
            ld = lambda k: xu_ref[k, pl.ds(j, 64, stride=4), 0:LW[k]]
            if k == 0:
                w = ld(0)
            elif k == 3:
                w = ld(3)
                w = jnp.where(lo, jnp.concatenate([w, w], axis=1), ld(2))
            else:
                w = jnp.where(lo, ld(k), ld(k - 1))
            w = pltpu.roll(w, 64, 1)
            dk = lam_ref[10, 0:1, 128 * k:128 * k + 128]
        for par in range(2):
            jj = 2 * j + par
            b = o[64 * jj:64 * jj + 64]
            if t >= 3:
                xv = pltpu.bitcast((w << 16) if par == 0 else (w & jnp.uint32(0xFFFF0000)), F32)
                b = jnp.where(lo, b, b + xv * dk) if t == 3 else b + xv * dk
            stage_ref[t, pl.ds(jj, 64, stride=8), :] = b
        yield


def _kernel(xa_hbm, wqkv_hbm, wo_hbm, xb_hbm, lre_hbm, lim_hbm, bre_hbm, bim_hbm, cre_hbm, cim_hbm,
            ldt_hbm, dsk_hbm, out_ref,
            xa_ref, xb_ref, wqkv_ref, wo_ref, cre_ref, cim_ref, lre_ref, lim_ref, ldt_ref, dsk_ref, isem, xsem,
            wt_ref, wot_ref, bcat_ref, ccat_ref, lam_ref, tmp_ref, tmpo_ref, tmpo2_ref, hc_ref,
            xau_ref, xap_ref, xbu_ref, xbp_ref, bu_ref, q_ref, k_ref, v_ref, prev_ref, kx_ref, vx_ref, p_ref, e_ref, ot_ref, h_ref, oa_ref, oy_ref,
            stage_ref, osem):
    i = pl.program_id(0)
    slot = i % 2
    qkv_ref, ext_ref = (q_ref, k_ref, v_ref), (kx_ref, vx_ref)

    def out_copy(blk, sl, k):
        return pltpu.make_async_copy(
            stage_ref.at[sl, k], out_ref.at[pl.ds(pl.multiple_of(blk * R, R), R), pl.ds(128 * k, 128)],
            osem.at[sl, k])

    def x_copies(b0, nb):
        cols = pl.ds(b0 * R, nb * R)
        return [pltpu.make_async_copy(xb_hbm.at[:, cols], xb_ref.at[:, cols], xsem.at[0, b0]),
                pltpu.make_async_copy(xa_hbm.at[:, cols], xa_ref.at[:, cols], xsem.at[1, b0])]

    cp = lambda n, src, dst: pltpu.make_async_copy(src, dst, isem.at[n])
    start = lambda g: [c.start() for c in g]
    wait = lambda g: [c.wait() for c in g]

    def body(first):
        cols = pl.ds(0, R) if first else pl.ds(pl.multiple_of(i * R, R), R)
        stage = stage_ref.at[0] if first else stage_ref.at[slot]

        zs = [0] * 7

        def wide(ref, r0, m):
            nt = ref.shape[0]
            return jnp.concatenate([ref[k, pl.ds(r0, m), 0:(LW[k] if nt == 4 else 128)] for k in range(nt)], axis=1)

        def bu_piece(n):
            def f():
                bu_ref[:, 128 * n:128 * n + 128] = lax.dot_general(
                    wide(xbp_ref, zs[n], R), bcat_ref[128 * n:128 * n + 128, :], NT, preferred_element_type=F32)
            return f

        def t_piece(dst, d0, lhs, r0, m, rhs):
            def f():
                for j in range(4):
                    dst[d0:d0 + m, 128 * j:128 * j + 128] = lax.dot_general(
                        wide(lhs, zs[j] + r0, m), wide(rhs, zs[(r0 // m) % 7] + 128 * j, 128), NT,
                        preferred_element_type=F32)
            return f

        qkv_piece = lambda r0, m: t_piece(qkv_ref[r0 // D], r0 % D, wt_ref, r0, m, xap_ref)
        y_piece = lambda r0, m: t_piece(oy_ref, r0, ccat_ref, r0, m, h_ref)

        def a_piece(r0, m):
            def f():
                for j in range(4):
                    oa_ref[r0:r0 + m, 128 * j:128 * j + 128] = jnp.dot(
                        wide(wot_ref, zs[j] + r0, m), ot_ref[j].astype(BF16), preferred_element_type=F32)
            return f

        region = lambda f: f()
        ext = lambda part, hg: _extend(qkv_ref, prev_ref, ext_ref[part], part, hg, first)
        scan = lambda k: _scan(bu_ref, lam_ref, hc_ref, h_ref, e_ref, k, first)
        logits = lambda hg: _logits(qkv_ref, ext_ref[0], p_ref, hg, first)
        qp, kp, vp = ([qkv_piece(n * D + r, PM) for r in range(0, D, PM)] for n in range(3))
        bp = [bu_piece(n) for n in range(7)]
        if first:
            xb0, xa0 = x_copies(0, 1)
            g0 = [xb0]
            for k in range(4):
                n = LW[k]
                g0.append(cp(2 * k, bre_hbm.at[128 * k:128 * k + n], bcat_ref.at[256 * k:256 * k + n]))
                g0.append(cp(2 * k + 1, bim_hbm.at[128 * k:128 * k + n], bcat_ref.at[256 * k + n:256 * k + 2 * n]))
            gw = [cp(8, wqkv_hbm, wqkv_ref), xa0,
                  cp(9, lre_hbm, lre_ref), cp(10, lim_hbm, lim_ref), cp(11, ldt_hbm, ldt_ref),
                  cp(12, dsk_hbm, dsk_ref)]
            gs = [cp(13, cre_hbm, cre_ref), cp(14, cim_hbm, cim_ref), cp(15, wo_hbm, wo_ref)]
            start(g0)
            wait(g0)
            start(gw)
            _permute_rows(xb_ref.at[:, cols], xbu_ref, xbp_ref)
            for piece in bp[:4]:
                piece()
            wait(gw)
            start(gs)
            for piece in bp[4:]:
                piece()
            _prep_wqkv(wqkv_ref, wt_ref, tmp_ref)
            _permute_rows(xa_ref.at[:, cols], xau_ref, xap_ref)
            coef = _prep_lam(lre_ref, lim_ref, ldt_ref, dsk_ref, lam_ref)
            wait(gs)
            start(x_copies(1, NB - 1))
            _mix(kp + qp, _chain(scan(0), scan(1), scan(2), ext(0, 0), ext(0, 1)), 54 + 56)
            region(lambda: _mix(vp, _chain(logits(0)), 32))
            _prep_c(coef, cre_ref, cim_ref, ccat_ref)
            _prep_wo(wo_ref, wot_ref, tmpo_ref, tmpo2_ref)
            for _ in _chain(scan(3), ext(1, 0), ext(1, 1), logits(2)):
                pass
        else:
            _permute_rows(xb_ref.at[:, cols], xbu_ref, xbp_ref)
            _mix(kp + qp, _chain(ext(0, 0), ext(0, 1)), 56, skip=1)
            region(lambda: _mix(bp[:3], logits(0), 32))
            region(lambda: _mix(bp[3:], _chain(logits(2), scan(0)), 50))
            region(lambda: _mix(vp, _chain(scan(1), scan(2), scan(3), ext(1, 0)), 54 + 28))
        yp = [y_piece(r, 64) for r in range(0, D, 64)]
        region(lambda: _mix(yp[:4], _chain(iter(()) if first else ext(1, 1), _values(ext_ref[1], p_ref, ot_ref, 0)),
                            28 + (0 if first else 28)))
        region(lambda: _mix(yp[4:], _values(ext_ref[1], p_ref, ot_ref, 2), 28))
        if first:
            wait(x_copies(1, NB - 1))
        st = lambda t: _store_tile(oa_ref, oy_ref, xbu_ref, lam_ref, stage, t)
        _mix([a_piece(384, 64), a_piece(0, 128), a_piece(128, 128), a_piece(256, 128)],
             _chain(st(4), st(5), st(6), st(3)), 16)
        start([out_copy(i, slot, k) for k in (3, 4, 5, 6)])
        nxt = pl.ds(pl.multiple_of(jnp.minimum(i + 1, NB - 1) * R, R), R)
        _permute_rows(xa_ref.at[:, nxt], xau_ref, xap_ref)
        for _ in _chain(st(0), st(1), st(2)):
            pass

    @pl.when(i >= 2)
    def _():
        wait([out_copy(i - 2, slot, k) for k in range(7)])

    pl.when(i == 0)(functools.partial(body, True))
    pl.when(i > 0)(functools.partial(body, False))
    start([out_copy(i, slot, k) for k in (0, 1, 2)])

    @pl.when(i == NB - 1)
    def _():
        wait([out_copy(i - 1, 1 - slot, k) for k in range(7)])
        wait([out_copy(i, slot, k) for k in range(7)])


def _call(A_x, A_wqkv, A_wo, B_x, lre, lim, bre, bim, cre, cim, ldt, dsk, interpret=False):
    hbm = pl.BlockSpec(memory_space=pltpu.HBM)
    V = pltpu.VMEM
    out = pl.pallas_call(
        _kernel,
        grid=(NB,),
        in_specs=[hbm] * 12,
        out_specs=hbm,
        out_shape=jax.ShapeDtypeStruct((S, 2 * D), F32),
        scratch_shapes=[
            V((D, S), BF16), V((D, S), BF16),
            V((D, 3 * D), BF16), V((D, D), BF16), V((D, D), BF16), V((D, D), BF16),
            V((D,), BF16), V((D,), BF16), V((D,), BF16), V((D,), BF16),
            pltpu.SemaphoreType.DMA((16,)), pltpu.SemaphoreType.DMA((2, 2)),
            V((4, 3 * D, 128), BF16), V((4, D, 128), BF16), V((2 * D, D), BF16), V((7, D, 128), BF16),
            V((11, 8, 512), F32), V((4, 3 * D, 128), F32), V((4, D, 128), F32), V((D, D), F32),
            V((2, 8, 512), F32),
            V((4, R // 2, 128), U32), V((4, R, 128), BF16), V((4, R // 2, 128), U32), V((4, R, 128), BF16),
            V((R, 2 * D), F32), V((D, R), F32), V((D, R), F32), V((D, R), F32), V((2, D, R), F32), V((11, D, 128), F32), V((11, D, 128), F32), V((2, 32, 8, 128), F32),
            V((4, 2, 72, 128), F32), V((4, D, 128), F32), V((7, R, 128), BF16), V((D, R), F32), V((D, R), F32),
            V((2, 7, R, 128), F32), pltpu.SemaphoreType.DMA((2, 7)),
        ],
        compiler_params=pltpu.CompilerParams(dimension_semantics=("arbitrary",), vmem_limit_bytes=100 * 2**20, flags={"XLA_TPU_FORCE_LP_LLO_SCHEDULER": True}),
        interpret=interpret,
        name="fused",
    )(A_x.reshape(S, D).T, A_wqkv, A_wo, B_x.reshape(S, D).T, lre, lim, bre, bim, cre, cim, ldt, dsk)
    return out.reshape(1, S, 2 * D)


@jax.jit
def pallas_concat_heads__sliding_local_dilated__ssm_conv_s5__prompt_kernel(
    A_x, A_wqkv, A_wo, B_x, B_Lambda_re, B_Lambda_im, B_B_re, B_B_im, B_C_re, B_C_im, B_log_dt, B_Dskip,
):
    return _call(A_x, A_wqkv, A_wo, B_x, B_Lambda_re, B_Lambda_im, B_B_re, B_B_im, B_C_re, B_C_im,
                 B_log_dt, B_Dskip)
```
